```python
import os as _os
_os.environ.setdefault("JAX_PLATFORMS", "cpu")
import jax
import jax.numpy as jnp

def _softmax(x, axis=-1):
    return jax.nn.softmax(x, axis=axis)
def _gelu(x):
    return jax.nn.gelu(x, approximate=True)
def _silu(x):
    return jax.nn.silu(x)
def _sigmoid(x):
    return jax.nn.sigmoid(x)
def _layernorm(x, axis=-1, eps=1e-5):
    m = jnp.mean(x, axis=axis, keepdims=True)
    v = jnp.var(x, axis=axis, keepdims=True)
    return (x - m) / jnp.sqrt(v + eps)
def _scatter_add(tgt, idx, src, axis=0):
    return tgt.at[idx].add(src)
def _segment_sum(src, seg, n):
    return jax.ops.segment_sum(src, seg, n)
class _Rng:
    def __init__(self, key):
        self._k = key
    def _next(self):
        self._k, sub = jax.random.split(self._k)
        return sub
    def normal(self, shape):
        return jax.random.normal(self._next(), shape, dtype=jnp.bfloat16)
    def randint(self, lo, hi, shape):
        return jax.random.randint(self._next(), shape, lo, hi, dtype=jnp.int32)
    def uniform(self, shape, lo=0.0, hi=1.0):
        return jax.random.uniform(self._next(), shape, jnp.bfloat16, lo, hi)
    def permutation(self, n):
        return jax.random.permutation(self._next(), n)


kernel_name = 'standalone__mha_softmax__sampling'

def setup_inputs():
    _rng = _Rng(jax.random.key(int.from_bytes(__import__("os").urandom(4), "little")))
    _w = (lambda a: (lambda t: t.astype(jnp.bfloat16) if jnp.issubdtype(t.dtype, jnp.floating) else t)(jnp.asarray(a)))
    B, H, Sq, Sk, D = 8, 32, 32, 2048, 128
    return {
        "q": _w((lambda *s: _rng.normal(s) * 0.4)(B, H, Sq, D)),
        "k": _w((lambda *s: _rng.normal(s) * 0.4)(B, H, Sk, D)),
        "v": _w((lambda *s: _rng.normal(s) * 0.05)(B, H, Sk, D)),
    }

def reference(q, k, v):
    scale = q.shape[-1] ** -0.5
    scores = jnp.einsum("bhqd,bhkd->bhqk", q, k) * scale
    p = _softmax(scores, axis=-1)
    return jnp.einsum("bhqk,bhkd->bhqd", p, v)
```

```python
import math

import jax
import jax.numpy as jnp
from jax import lax
import jax.experimental.pallas as pl
import jax.experimental.pallas.tpu as pltpu

_G = 8
_HS = 2
_ROWS = 128
_WRITE_STREAMS = 8


@jax.jit
def pallas_standalone__mha_softmax__sampling_kernel(
    q: jax.Array,
    k: jax.Array,
    v: jax.Array,
):
    B, H, Sq, D = q.shape
    Sk = k.shape[2]
    N = B * H
    G, HS, ROWS = _G, _HS, _ROWS
    assert N % (G * HS) == 0 and Sk % ROWS == 0
    num_blocks = N // (G * HS)
    num_groups = N // G
    exp2_scale = (D ** -0.5) * math.log2(math.e)

    k_off, v_off, q_off, head_rows = 0, Sk, 2 * Sk, 2 * Sk + Sq

    schedule = [("q", t * (G // 2), 0) for t in range(2)]
    for j in range(Sk // ROWS):
        for g in range(G):
            schedule += [("k", g, j * ROWS), ("v", g, j * ROWS)]
    cut0 = len(schedule) // 2
    cut1 = 3 * len(schedule) // 4

    out_rows = N * Sq
    done_rows = (num_blocks - 1) * G * HS * Sq

    def kernel(q_hbm, k_hbm, v_hbm, o_hbm, buf, p_buf, inv_buf, o_buf, sems, o_sem):
        def start_loads(group, slot, lo, hi):
            block, r = group // HS, group % HS
            for n in range(lo, hi):
                what, g, row = schedule[n]
                if what == "q":
                    src = q_hbm.at[block, pl.ds(g, G // 2), r]
                    dst = buf.at[slot, pl.ds(g, G // 2), pl.ds(q_off, Sq)]
                else:
                    hbm, off = (k_hbm, k_off) if what == "k" else (v_hbm, v_off)
                    src = hbm.at[block, g, r, pl.ds(row, ROWS)]
                    dst = buf.at[slot, g, pl.ds(off + row, ROWS)]
                pltpu.make_async_copy(src, dst, sems.at[slot]).start(priority=n % 2)

        def wait_loads(slot):
            pltpu.make_async_copy(buf.at[slot], buf.at[slot], sems.at[slot]).wait()

        def start_store(row, rows, priority):
            pltpu.make_async_copy(
                o_buf.at[pl.ds(row, rows)], o_hbm.at[pl.ds(row, rows)], o_sem
            ).start(priority=priority)

        def softmax_stage(slot):
            for g in range(G):
                s = lax.dot_general(
                    buf[slot, g, pl.ds(q_off, Sq)],
                    buf[slot, g, pl.ds(k_off, Sk)],
                    (((1,), (1,)), ((), ())),
                    preferred_element_type=jnp.float32,
                )
                m = jnp.max(s, axis=-1, keepdims=True)
                p = jnp.exp2((s - m) * exp2_scale)
                l = jnp.sum(p, axis=-1, keepdims=True)
                p_buf[g] = p.astype(p_buf.dtype)
                inv_buf[g] = jnp.broadcast_to(1.0 / l, (Sq, D))

        def value_stage(group, slot):
            block, r = group // HS, group % HS
            for g in range(G):
                o = jnp.dot(
                    p_buf[g],
                    buf[slot, g, pl.ds(v_off, Sk)],
                    preferred_element_type=jnp.float32,
                )
                row = pl.multiple_of(((block * G + g) * HS + r) * Sq, Sq)
                o_buf[pl.ds(row, Sq)] = (o * inv_buf[g]).astype(o_buf.dtype)

        start_loads(0, 0, 0, len(schedule))

        def step(group, _):
            slot = group % 2
            start_loads(group + 1, 1 - slot, 0, cut0)
            wait_loads(slot)
            softmax_stage(slot)
            start_loads(group + 1, 1 - slot, cut0, cut1)
            value_stage(group, slot)
            start_loads(group + 1, 1 - slot, cut1, len(schedule))

        lax.fori_loop(0, num_groups - 1, step, None)

        last = num_groups - 1
        wait_loads(last % 2)
        per_stream = out_rows // _WRITE_STREAMS
        n = 0
        for j in range(0, per_stream, ROWS):
            for stream in range(_WRITE_STREAMS):
                row = stream * per_stream + j
                if row < done_rows:
                    start_store(row, min(ROWS, done_rows - row), n % 2)
                    n += 1
        softmax_stage(last % 2)
        value_stage(last, last % 2)
        half = (out_rows - done_rows) // 2
        start_store(done_rows, half, 0)
        start_store(done_rows + half, half, 1)
        pltpu.make_async_copy(o_buf, o_hbm, o_sem).wait()

    out = pl.pallas_call(
        kernel,
        in_specs=[pl.BlockSpec(memory_space=pl.ANY)] * 3,
        out_specs=pl.BlockSpec(memory_space=pl.ANY),
        out_shape=jax.ShapeDtypeStruct((out_rows, D), q.dtype),
        scratch_shapes=[
            pltpu.VMEM((2, G, head_rows, D), k.dtype),
            pltpu.VMEM((G, Sq, Sk), v.dtype),
            pltpu.VMEM((G, Sq, D), jnp.float32),
            pltpu.VMEM((out_rows, D), q.dtype),
            pltpu.SemaphoreType.DMA((2,)),
            pltpu.SemaphoreType.DMA(()),
        ],
        compiler_params=pltpu.CompilerParams(vmem_limit_bytes=64 * 1024 * 1024),
    )(
        q.reshape(num_blocks, G, HS, Sq, D),
        k.reshape(num_blocks, G, HS, Sk, D),
        v.reshape(num_blocks, G, HS, Sk, D),
    )
    return out.reshape(B, H, Sq, D)
```

```python
import math

import jax
import jax.numpy as jnp
from jax import lax
import jax.experimental.pallas as pl
import jax.experimental.pallas.tpu as pltpu

_G = 8
_HS = 2
_HEAD_ORDER = (0, 3, 2, 1, 4, 6, 7, 5)
_ROWS = 128
_LATE_CHUNKS = 3
_WRITE_STREAMS = 8


@jax.jit
def pallas_standalone__mha_softmax__sampling_kernel(
    q: jax.Array,
    k: jax.Array,
    v: jax.Array,
):
    B, H, Sq, D = q.shape
    Sk = k.shape[2]
    N = B * H
    G, HS, ROWS = _G, _HS, _ROWS
    assert N % (G * HS) == 0 and Sk % ROWS == 0
    assert sorted(_HEAD_ORDER) == list(range(G))
    num_blocks = N // (G * HS)
    num_groups = N // G
    chunks = Sk // ROWS
    halves = (range(0, G // 2), range(G // 2, G))
    exp2_scale = (D ** -0.5) * math.log2(math.e)

    k_off, v_off, q_off, head_rows = 0, Sk, 2 * Sk, 2 * Sk + Sq

    out_rows = N * Sq
    done_rows = (num_blocks - 1) * G * HS * Sq

    def kernel(
        q_hbm, k_hbm, v_hbm, o_hbm,
        buf, p_buf, inv_buf, o_buf, slot_sems, last_sems, o_sem,
    ):
        def q_copy(group, half, sem):
            heads = pl.ds(half.start, len(half))
            return pltpu.make_async_copy(
                q_hbm.at[group // HS, heads, group % HS],
                buf.at[group % 2, heads, pl.ds(q_off, Sq)],
                sem,
            )

        def kv_copies(group, heads, lo, hi, sem, wait=False):
            def chunk(j, _):
                row = pl.multiple_of(j * ROWS, ROWS)
                for g in _HEAD_ORDER:
                    if g not in heads:
                        continue
                    for priority, (hbm, off) in enumerate(
                        ((k_hbm, k_off), (v_hbm, v_off))
                    ):
                        copy = pltpu.make_async_copy(
                            hbm.at[group // HS, g, group % HS, pl.ds(row, ROWS)],
                            buf.at[group % 2, g, pl.ds(off + row, ROWS)],
                            sem,
                        )
                        if wait:
                            copy.wait()
                        else:
                            copy.start(priority=priority)

            lax.fori_loop(lo, hi, chunk, None)

        def wait_filled(ref, sem):
            pltpu.make_async_copy(ref, ref, sem).wait()

        def softmax_stage(group, heads):
            slot = group % 2
            for g in heads:
                s = lax.dot_general(
                    buf[slot, g, pl.ds(q_off, Sq)],
                    buf[slot, g, pl.ds(k_off, Sk)],
                    (((1,), (1,)), ((), ())),
                    preferred_element_type=jnp.float32,
                )
                m = jnp.max(s, axis=-1, keepdims=True)
                p = jnp.exp2((s - m) * exp2_scale)
                l = jnp.sum(p, axis=-1, keepdims=True)
                p_buf[g] = p.astype(p_buf.dtype)
                inv_buf[g] = jnp.broadcast_to(1.0 / l, (Sq, D))

        def value_stage(group, heads):
            slot = group % 2
            for g in heads:
                o = jnp.dot(
                    p_buf[g],
                    buf[slot, g, pl.ds(v_off, Sk)],
                    preferred_element_type=jnp.float32,
                )
                head = ((group // HS) * G + g) * HS + group % HS
                o_buf[pl.ds(pl.multiple_of(head * Sq, Sq), Sq)] = (
                    o * inv_buf[g]
                ).astype(o_buf.dtype)

        def step(group, prefetch):
            prefetch[0]()
            wait_filled(buf.at[group % 2], slot_sems.at[group % 2])
            softmax_stage(group, halves[0])
            prefetch[1]()
            softmax_stage(group, halves[1])
            prefetch[2]()
            value_stage(group, range(G))
            prefetch[3]()

        def start_group(group, lo, hi):
            sem = slot_sems.at[group % 2]
            if lo == 0:
                for priority, half in enumerate(halves):
                    q_copy(group, half, sem).start(priority=priority)
            kv_copies(group, range(G), lo, hi, sem)

        def start_store(row, rows, priority):
            pltpu.make_async_copy(
                o_buf.at[pl.ds(row, rows)], o_hbm.at[pl.ds(row, rows)], o_sem
            ).start(priority=priority)

        cuts = (0, 7 * chunks // 16, 10 * chunks // 16, 13 * chunks // 16, chunks)

        def steady_step(group, _):
            step(group, [
                lambda t=t: start_group(group + 1, cuts[t], cuts[t + 1])
                for t in range(4)
            ])

        start_group(0, 0, chunks)
        lax.fori_loop(0, num_groups - 2, steady_step, None)

        last = num_groups - 1
        late = max(chunks - _LATE_CHUNKS, 0)
        mid = min(chunks // 2, late)

        def start_first_half():
            q_copy(last, halves[0], last_sems.at[0]).start(priority=1)
            kv_copies(last, halves[0], 0, chunks, last_sems.at[0])

        def start_second_half():
            q_copy(last, halves[1], last_sems.at[1]).start(priority=1)
            kv_copies(last, halves[1], 0, mid, last_sems.at[1])

        step(last - 1, [
            start_first_half,
            start_second_half,
            lambda: kv_copies(last, halves[1], mid, late, last_sems.at[1]),
            lambda: kv_copies(last, halves[1], late, chunks, last_sems.at[2]),
        ])

        wait_filled(buf.at[last % 2, pl.ds(0, G // 2)], last_sems.at[0])
        softmax_stage(last, halves[0])
        value_stage(last, halves[0])

        q_copy(last, halves[1], last_sems.at[1]).wait()
        kv_copies(last, halves[1], 0, late, last_sems.at[1], wait=True)
        per_stream = out_rows // _WRITE_STREAMS
        n = 0
        for j in range(0, per_stream, ROWS):
            for stream in range(_WRITE_STREAMS):
                row = stream * per_stream + j
                if row < done_rows:
                    rows = min(ROWS, per_stream - j, done_rows - row)
                    start_store(row, rows, n % 2)
                    n += 1
        kv_copies(last, halves[1], late, chunks, last_sems.at[2], wait=True)
        softmax_stage(last, halves[1])
        value_stage(last, halves[1])

        rest = (out_rows - done_rows) // 2
        start_store(done_rows, rest, 0)
        start_store(done_rows + rest, rest, 1)
        pltpu.make_async_copy(o_buf, o_hbm, o_sem).wait()

    out = pl.pallas_call(
        kernel,
        in_specs=[pl.BlockSpec(memory_space=pl.ANY)] * 3,
        out_specs=pl.BlockSpec(memory_space=pl.ANY),
        out_shape=jax.ShapeDtypeStruct((out_rows, D), q.dtype),
        scratch_shapes=[
            pltpu.VMEM((2, G, head_rows, D), k.dtype),
            pltpu.VMEM((G, Sq, Sk), v.dtype),
            pltpu.VMEM((G, Sq, D), jnp.float32),
            pltpu.VMEM((out_rows, D), q.dtype),
            pltpu.SemaphoreType.DMA((2,)),
            pltpu.SemaphoreType.DMA((3,)),
            pltpu.SemaphoreType.DMA(()),
        ],
        compiler_params=pltpu.CompilerParams(vmem_limit_bytes=64 * 1024 * 1024),
    )(
        q.reshape(num_blocks, G, HS, Sq, D),
        k.reshape(num_blocks, G, HS, Sk, D),
        v.reshape(num_blocks, G, HS, Sk, D),
    )
    return out.reshape(B, H, Sq, D)
```
